```python
import os as _os
_os.environ.setdefault("JAX_PLATFORMS", "cpu")
import jax
import jax.numpy as jnp

def _softmax(x, axis=-1):
    return jax.nn.softmax(x, axis=axis)
def _gelu(x):
    return jax.nn.gelu(x, approximate=True)
def _silu(x):
    return jax.nn.silu(x)
def _sigmoid(x):
    return jax.nn.sigmoid(x)
def _layernorm(x, axis=-1, eps=1e-5):
    m = jnp.mean(x, axis=axis, keepdims=True)
    v = jnp.var(x, axis=axis, keepdims=True)
    return (x - m) / jnp.sqrt(v + eps)
def _scatter_add(tgt, idx, src, axis=0):
    return tgt.at[idx].add(src)
def _segment_sum(src, seg, n):
    return jax.ops.segment_sum(src, seg, n)
class _Rng:
    def __init__(self, key):
        self._k = key
    def _next(self):
        self._k, sub = jax.random.split(self._k)
        return sub
    def normal(self, shape):
        return jax.random.normal(self._next(), shape, dtype=jnp.bfloat16)
    def randint(self, lo, hi, shape):
        return jax.random.randint(self._next(), shape, lo, hi, dtype=jnp.int32)
    def uniform(self, shape, lo=0.0, hi=1.0):
        return jax.random.uniform(self._next(), shape, jnp.bfloat16, lo, hi)
    def permutation(self, n):
        return jax.random.permutation(self._next(), n)


kernel_name = 'sequential_preLN__softmax_full_mha__mixer_channel_mlp__prompt'

def setup_inputs():
    _rng = _Rng(jax.random.key(int.from_bytes(__import__("os").urandom(4), "little")))
    _w = (lambda a: (lambda t: t.astype(jnp.bfloat16) if jnp.issubdtype(t.dtype, jnp.floating) else t)(jnp.asarray(a)))
    def _A_setup():
        B, S, D = 1, 2048, 1024
        return {
            "x": _w((lambda *s: _rng.normal(s) * 0.05)(B, S, D)),
            "wqkv": _w((lambda *s: _rng.normal(s) * 0.05)(D, 3 * D)),
            "wo": _w((lambda *s: _rng.normal(s) * 0.05)(D, D)),
        }
    _A_in = _A_setup()

    def _B_setup():
        B, S, D, F = 1, 2048, 1024, 3584
        return {
            "x": _w((lambda *s: _rng.normal(s) * 0.05)(B, S, D)),
            "w1": _w((lambda *s: _rng.normal(s) * 0.8)(D, F) * (D ** -0.5)),
            "b1": _w((lambda *s: _rng.normal(s) * 0.8)(F)),
            "w2": _w((lambda *s: _rng.normal(s) * 0.8)(F, D) * (F ** -0.5)),
            "b2": _w((lambda *s: _rng.normal(s) * 0.05)(D)),
        }
    _B_in = _B_setup()

    return {
        "A_x": _A_in["x"],
        "A_wqkv": _A_in["wqkv"],
        "A_wo": _A_in["wo"],
        "B_x": _B_in["x"],
        "B_w1": _B_in["w1"],
        "B_b1": _B_in["b1"],
        "B_w2": _B_in["w2"],
        "B_b2": _B_in["b2"],
    }

def reference(A_x, A_wqkv, A_wo, B_x, B_w1, B_b1, B_w2, B_b2):
    def _A_ref(x, wqkv, wo):
        B, S, D = x.shape
        H = 32; Dh = D // H
        qkv = (lambda x, *d: x.transpose(*d))((x @ wqkv).reshape(B, S, 3, H, Dh), 2, 0, 3, 1, 4)
        q, k, v = qkv[0], qkv[1], qkv[2]
        scale = Dh ** -0.5
        scores = jnp.einsum("bhqd,bhkd->bhqk", q, k) * scale
        p = _softmax(scores, axis=-1)
        o = jnp.einsum("bhqk,bhkd->bhqd", p, v)
        return (lambda x, *d: x.transpose(*d))(o, 0, 2, 1, 3).reshape(B, S, D) @ wo

    def _B_ref(x, w1, b1, w2, b2):
        y = _layernorm(x, axis=-1)
        h = _gelu(jnp.einsum("bsd,df->bsf", y, w1) + b1)
        return jnp.einsum("bsf,fd->bsd", h, w2) + b2

    x = A_x
    h = x + _A_ref(_layernorm(x, axis=-1), A_wqkv, A_wo)
    h2 = h + _B_ref(_layernorm(h, axis=-1), B_w1, B_b1, B_w2, B_b2)
    return h2
```

```python
import math

import jax
import jax.numpy as jnp
from jax import lax
import jax.experimental.pallas as pl
import jax.experimental.pallas.tpu as pltpu

S, D, F = 2048, 1024, 3584
H, DH = 32, 32
G = D // 128
HPG = 128 // DH
EPS = 1e-5

T = 256
NT = S // T
SUB = 512
NS = S // SUB
KC = 128
NC = S // KC
FC = 512
NF = F // FC
WC = 512
NW = 3 * D // WC

QSCALE = (DH ** -0.5) * math.log2(math.e)

SEM_X = 0
SEM_W = SEM_X + NT
SEM_WO = SEM_W + NW
SEM_W1 = SEM_WO + 1
SEM_W2 = SEM_W1 + 1
SEM_B1 = SEM_W2 + 1
SEM_B2 = SEM_B1 + 1
SEM_OUT = SEM_B2 + 1
NSEM = SEM_OUT + NT

f32 = jnp.float32
bf16 = jnp.bfloat16


def _layernorm(x):
    m = jnp.mean(x, axis=-1, keepdims=True)
    xc = x - m
    v = jnp.mean(xc * xc, axis=-1, keepdims=True)
    return xc * lax.rsqrt(v + EPS)


def _kernel(x_hbm, wqkv_hbm, wo_hbm, w1_hbm, b1_hbm, w2_hbm, b2_hbm, out_hbm,
            x_ref, wqkv_ref, wo_ref, w1_ref, b1_ref, w2_ref, b2_ref,
            ln_ref, q_ref, k_ref, vt_ref, s_ref, m_ref, ot_ref,
            y_ref, h_ref, o_stage, sems):

    def rows(t):
        if isinstance(t, int):
            return pl.ds(t * T, T)
        return pl.ds(pl.multiple_of(t * T, T), T)

    def x_copy(t):
        return pltpu.make_async_copy(x_hbm.at[rows(t), :], x_ref.at[rows(t), :], sems.at[SEM_X + t])

    def w_copy(n):
        return pltpu.make_async_copy(wqkv_hbm.at[:, pl.ds(n * WC, WC)],
                                     wqkv_ref.at[:, pl.ds(n * WC, WC)], sems.at[SEM_W + n])

    def out_copy(t):
        return pltpu.make_async_copy(o_stage.at[rows(t), :], out_hbm.at[rows(t), :],
                                     sems.at[SEM_OUT + t])

    wo_copy = pltpu.make_async_copy(wo_hbm, wo_ref, sems.at[SEM_WO])
    w1_copy = pltpu.make_async_copy(w1_hbm, w1_ref, sems.at[SEM_W1])
    w2_copy = pltpu.make_async_copy(w2_hbm, w2_ref, sems.at[SEM_W2])
    b1_copy = pltpu.make_async_copy(b1_hbm, b1_ref, sems.at[SEM_B1])
    b2_copy = pltpu.make_async_copy(b2_hbm, b2_ref, sems.at[SEM_B2])

    x_copy(0).start()
    for n in range(NW):
        w_copy(n).start()
    for t in range(1, NT):
        x_copy(t).start()

    def ln_tile(t):
        return _layernorm(x_ref[rows(t), :].astype(f32)).astype(bf16)

    def qkv_chunk(ln, t, n):
        z = jnp.dot(ln, wqkv_ref[:, n * WC:(n + 1) * WC], preferred_element_type=f32)
        which, off = divmod(n * WC, D)
        g0 = off // 128
        if which == 0:
            zb = (z * QSCALE).astype(bf16)
            for i in range(WC // 128):
                q_ref[g0 + i, rows(t), :] = zb[:, i * 128:(i + 1) * 128]
        elif which == 1:
            zb = z.astype(bf16)
            for i in range(WC // 128):
                k_ref[g0 + i, rows(t), :] = zb[:, i * 128:(i + 1) * 128]
        else:
            vt_ref[t, off:off + WC, :] = z.astype(bf16).T

    x_copy(0).wait()
    ln0 = ln_tile(0)
    for n in range(NW):
        w_copy(n).wait()
        qkv_chunk(ln0, 0, n)
    x_copy(1).wait()
    ln_ref[...] = ln_tile(1)

    wo_copy.start()
    w1_copy.start()
    w2_copy.start()
    b1_copy.start()
    b2_copy.start()

    def qkv_body(t, carry):
        @pl.when(t + 1 < NT)
        def _():
            x_copy(t + 1).wait()

        ln = ln_ref[...]
        for n in range(NW):
            qkv_chunk(ln, t, n)
            if n == 1:
                ln_ref[...] = ln_tile(jnp.minimum(t + 1, NT - 1))
        return carry

    lax.fori_loop(1, NT, qkv_body, 0)

    lane_head = lax.broadcasted_iota(jnp.int32, (SUB, 128), 1) // DH

    def q_masked(u, g, j):
        q = q_ref[g, u * SUB:(u + 1) * SUB, :]
        return jnp.where(lane_head == j, q, jnp.zeros_like(q))

    def a_chunk(qm, g, c, b, u, m):
        kc = k_ref[g, c * KC:(c + 1) * KC, :]
        s = lax.dot_general(kc, qm, (((1,), (1,)), ((), ())), preferred_element_type=f32)
        s_ref[b, u, c * KC:(c + 1) * KC, :] = s
        for r in range(KC // 8):
            sr = s[8 * r:8 * r + 8, :]
            m = sr if m is None else jnp.maximum(m, sr)
        return m

    def a_finish(b, u, m):
        m_ref[b, u] = jnp.broadcast_to(jnp.max(m, axis=0, keepdims=True), (8, SUB))

    def b_chunk(h, c, b, u, m, l, acc):
        s = s_ref[b, u, c * KC:(c + 1) * KC, :]
        p = jnp.exp2(s - m)
        for a in reversed(range(KC // 16)):
            pr = p[16 * a:16 * a + 8, :] + p[16 * a + 8:16 * a + 16, :]
            l = pr if l is None else l + pr
        per = T // KC
        hrows = pl.ds(h * DH, DH) if isinstance(h, int) else pl.ds(pl.multiple_of(h * DH, DH), DH)
        vt = vt_ref[c // per, hrows, (c % per) * KC:(c % per + 1) * KC]
        o = jnp.dot(vt, p.astype(bf16), preferred_element_type=f32)
        acc = o if acc is None else acc + o
        return l, acc

    def b_finish(h, u, l, acc):
        lsum = jnp.sum(l, axis=0, keepdims=True)
        o = (acc * (1.0 / lsum)).astype(bf16)
        hrows = pl.ds(h * DH, DH) if isinstance(h, int) else pl.ds(pl.multiple_of(h * DH, DH), DH)
        per = SUB // T
        for i in range(per):
            ot_ref[u * per + i, hrows, :] = o[:, i * T:(i + 1) * T]

    def attn_step(h, b, do_a, do_b):
        hn = h + 1
        for u in range(NS):
            if do_a:
                qm = q_masked(u, hn // HPG, hn % HPG)
            if do_b:
                mrow = m_ref[b, u, 0:1, :]
            m = l = acc = None
            for c in range(NC):
                if do_a:
                    m = a_chunk(qm, hn // HPG, c, 1 - b, u, m)
                if do_b:
                    l, acc = b_chunk(h, c, b, u, mrow, l, acc)
            if do_a:
                a_finish(1 - b, u, m)
            if do_b:
                b_finish(h, u, l, acc)

    attn_step(-1, 1, True, False)

    def head_body(h, carry):
        @pl.when(h % 2 == 0)
        def _():
            attn_step(h, 0, True, True)

        @pl.when(h % 2 == 1)
        def _():
            attn_step(h, 1, True, True)
        return carry

    lax.fori_loop(0, H - 1, head_body, 0)
    attn_step(H - 1, (H - 1) % 2, False, True)

    wo_copy.wait()
    w1_copy.wait()
    w2_copy.wait()
    b1_copy.wait()
    b2_copy.wait()

    def wo_ln(t):
        o = ot_ref[t].T
        a = jnp.dot(o, wo_ref[...], preferred_element_type=f32)
        h = x_ref[rows(t), :].astype(f32) + a
        y = _layernorm(_layernorm(h))
        h_ref[...] = h
        y_ref[...] = y.astype(bf16)

    def mlp(t, next_t):
        y = y_ref[...]
        acc = h_ref[...] + b2_ref[...].astype(f32)

        def mm1(c):
            z = jnp.dot(y, w1_ref[:, c * FC:(c + 1) * FC], preferred_element_type=f32)
            z = z + b1_ref[:, c * FC:(c + 1) * FC].astype(f32)
            return jax.nn.gelu(z, approximate=True).astype(bf16)

        h1 = mm1(0)
        for c in range(NF):
            h1n = mm1(c + 1) if c + 1 < NF else None
            if c == 1 and next_t is not None:
                wo_ln(next_t)
            acc = acc + jnp.dot(h1, w2_ref[c * FC:(c + 1) * FC, :], preferred_element_type=f32)
            h1 = h1n
        o_stage[rows(t), :] = acc.astype(bf16)
        out_copy(t).start()

    wo_ln(0)

    def mlp_body(t, carry):
        mlp(t, t + 1)
        return carry

    lax.fori_loop(0, NT - 1, mlp_body, 0)
    mlp(NT - 1, None)

    for t in range(NT):
        out_copy(t).wait()


@jax.jit
def pallas_sequential_preLN__softmax_full_mha__mixer_channel_mlp__prompt_kernel(
    A_x: jax.Array,
    A_wqkv: jax.Array,
    A_wo: jax.Array,
    B_x: jax.Array,
    B_w1: jax.Array,
    B_b1: jax.Array,
    B_w2: jax.Array,
    B_b2: jax.Array,
):
    del B_x
    x = A_x.reshape(S, D)
    b1 = B_b1.reshape(1, F)
    b2 = B_b2.reshape(1, D)

    any_spec = pl.BlockSpec(memory_space=pl.ANY)
    out = pl.pallas_call(
        _kernel,
        out_shape=jax.ShapeDtypeStruct((S, D), bf16),
        in_specs=[any_spec] * 7,
        out_specs=any_spec,
        scratch_shapes=[
            pltpu.VMEM((S, D), bf16),
            pltpu.VMEM((D, 3 * D), bf16),
            pltpu.VMEM((D, D), bf16),
            pltpu.VMEM((D, F), bf16),
            pltpu.VMEM((1, F), bf16),
            pltpu.VMEM((F, D), bf16),
            pltpu.VMEM((1, D), bf16),
            pltpu.VMEM((T, D), bf16),
            pltpu.VMEM((G, S, 128), bf16),
            pltpu.VMEM((G, S, 128), bf16),
            pltpu.VMEM((NT, D, T), bf16),
            pltpu.VMEM((2, NS, S, SUB), f32),
            pltpu.VMEM((2, NS, 8, SUB), f32),
            pltpu.VMEM((NT, D, T), bf16),
            pltpu.VMEM((T, D), bf16),
            pltpu.VMEM((T, D), f32),
            pltpu.VMEM((S, D), bf16),
            pltpu.SemaphoreType.DMA((NSEM,)),
        ],
        compiler_params=pltpu.CompilerParams(vmem_limit_bytes=120 * 1024 * 1024),
    )(x, A_wqkv, A_wo, B_w1, b1, B_w2, b2)
    return out.reshape(1, S, D)
```

```python
import math

import jax
import jax.numpy as jnp
from jax import lax
import jax.experimental.pallas as pl
import jax.experimental.pallas.tpu as pltpu

S, D, F = 2048, 1024, 3584
H, DH = 32, 32
G = D // 128
HPG = 128 // DH
EPS = 1e-5

T = 256
NT = S // T
T1 = 512
NT1 = S // T1
RB = 16
SUB = 512
NS = S // SUB
KC = 128
NC = S // KC
HB = 2
FC = 256
NF = F // FC
KP = D - 128

W_PIECES = ((0, 256), (256, 256), (512, 512), (2048, 512), (1024, 512), (2560, 512), (1536, 512))
W_CHUNKS = ((2048, 512), (2560, 512), (0, 512), (512, 512), (1024, 512), (1536, 512))
X_PIECES = ((0, 256), (256, 256)) + tuple((i * T1, T1) for i in range(1, NT1))

QSCALE = (DH ** -0.5) * math.log2(math.e)

SEM_X = 0
SEM_W = SEM_X + len(X_PIECES)
SEM_WO = SEM_W + len(W_PIECES)
SEM_MLP = SEM_WO + 1
SEM_OUT = SEM_MLP + 1
NSEM = SEM_OUT + 1
TO = 64

BIAS_PAD = 32768

f32 = jnp.float32
bf16 = jnp.bfloat16


def _layernorm(x):
    m = jnp.mean(x, axis=-1, keepdims=True)
    xc = x - m
    v = jnp.mean(xc * xc, axis=-1, keepdims=True)
    return xc * lax.rsqrt(v + EPS)


def _layernorm_centered(z):
    m = jnp.mean(z, axis=-1, keepdims=True)
    v = jnp.mean(z * z, axis=-1, keepdims=True) - m * m
    return (z - m) * lax.rsqrt(v + EPS)


def _ds(start, size, align):
    if isinstance(start, int):
        return pl.ds(start, size)
    return pl.ds(pl.multiple_of(start, align), size)


def _interleave(main, side, ratio):
    for _ in main:
        for _ in range(ratio):
            next(side, None)
    _drain(side)


def _drain(gen):
    for _ in gen:
        pass


def _chain(*gens):
    for g in gens:
        for _ in g:
            yield


def _kernel(x_hbm, wqkv_hbm, wo_hbm, w1_hbm, b1_hbm, w2_hbm, b2_hbm, out_hbm,
            x_ref, wqkv_ref, wo_ref, w1_ref, b1_ref, w2_ref, b2_ref,
            ln_ref, q_ref, k_ref, vt_ref, s_ref, m_ref, ot_ref,
            y_ref, h_ref, o_stage, sems):

    def rows(t):
        return _ds(t * T, T, T)

    def x_copy(i):
        if isinstance(i, int):
            r = pl.ds(*X_PIECES[i])
        else:
            r = _ds((i - 1) * T1, T1, T1)
        return pltpu.make_async_copy(x_hbm.at[r, :], x_ref.at[r, :], sems.at[SEM_X + i])

    def w_copy(i):
        c = pl.ds(*W_PIECES[i])
        return pltpu.make_async_copy(wqkv_hbm.at[:, c], wqkv_ref.at[:, c], sems.at[SEM_W + i])

    def out_copy(i):
        r = _ds(i * TO, TO, TO)
        return pltpu.make_async_copy(o_stage.at[r, :], out_hbm.at[r, :], sems.at[SEM_OUT])

    wo_copy = pltpu.make_async_copy(wo_hbm, wo_ref, sems.at[SEM_WO])
    w1_copy = pltpu.make_async_copy(w1_hbm, w1_ref, sems.at[SEM_MLP])
    w2_copy = pltpu.make_async_copy(w2_hbm, w2_ref, sems.at[SEM_MLP])
    b1_copy = pltpu.make_async_copy(b1_hbm, b1_ref.at[pl.ds(0, F)], sems.at[SEM_MLP])
    b2_copy = pltpu.make_async_copy(b2_hbm, b2_ref.at[pl.ds(0, D)], sems.at[SEM_MLP])

    x_copy(0).start()
    w_copy(0).start()
    x_copy(1).start()
    for i in range(1, len(W_PIECES)):
        w_copy(i).start()
    for i in range(2, len(X_PIECES)):
        x_copy(i).start()
    wo_copy.start()
    w1_copy.start()
    w2_copy.start()
    b1_copy.start()
    b2_copy.start()

    def ln1_gen(row0, off, n):
        for r in range(0, n, RB):
            xb = x_ref[_ds(row0 + r, RB, RB), :].astype(f32)
            ln_ref[off + r:off + r + RB, :] = _layernorm(xb).astype(bf16)
            yield

    def ln1(row0, off, n):
        _drain(ln1_gen(row0, off, n))

    def qkv_dot(ln, row0, col0, ncol):
        nrow = ln.shape[0]
        z = jnp.dot(ln, wqkv_ref[:, col0:col0 + ncol], preferred_element_type=f32)
        which, off = divmod(col0, D)
        r = _ds(row0, nrow, nrow)
        if which == 0:
            zb = (z * QSCALE).astype(bf16)
            for i in range(ncol // 128):
                q_ref[off // 128 + i, r, :] = zb[:, i * 128:(i + 1) * 128]
        elif which == 1:
            zb = z.astype(bf16)
            for i in range(ncol // 128):
                k_ref[off // 128 + i, r, :] = zb[:, i * 128:(i + 1) * 128]
        else:
            zt = z.astype(bf16).T
            for i in range(nrow // T):
                vt_ref[row0 // T + i, off:off + ncol, :] = zt[:, i * T:(i + 1) * T]

    x_copy(0).wait()
    ln1(0, 0, 256)
    w_copy(0).wait()
    qkv_dot(ln_ref[0:256, :], 0, *W_PIECES[0])
    x_copy(1).wait()
    ln1(256, 256, 256)
    qkv_dot(ln_ref[256:512, :], 256, *W_PIECES[0])
    w_copy(1).wait()
    qkv_dot(ln_ref[...], 0, *W_PIECES[1])
    w_copy(2).wait()
    qkv_dot(ln_ref[...], 0, *W_PIECES[2])
    w_copy(3).wait()
    w_copy(4).wait()
    qkv_dot(ln_ref[...], 0, *W_PIECES[3])
    qkv_dot(ln_ref[...], 0, *W_PIECES[4])
    w_copy(5).wait()
    w_copy(6).wait()
    x_copy(2).wait()
    ln0 = ln_ref[...]
    qkv_dot(ln0, 0, *W_PIECES[5])
    ln1(T1, 0, T1)
    qkv_dot(ln0, 0, *W_PIECES[6])

    def qkv_body(t, carry):
        @pl.when(t + 1 < NT1)
        def _():
            x_copy(t + 2).wait()

        ln = ln_ref[...]

        def chunks():
            for c0, nc in W_CHUNKS:
                qkv_dot(ln, t * T1, c0, nc)
                yield

        _interleave(chunks(), ln1_gen(jnp.minimum(t + 1, NT1 - 1) * T1, 0, T1), 7)
        return carry

    lax.fori_loop(1, NT1, qkv_body, 0)

    lane_head = lax.broadcasted_iota(jnp.int32, (SUB, 128), 1) // DH

    def attn_gen(hb, ha, hh, u):
        if ha is not None:
            ga = ha >> 2
            q = q_ref[ga, u * SUB:(u + 1) * SUB, :]
            qm = jnp.where(lane_head == (ha & 3), q, jnp.zeros_like(q))
        if hb is not None:
            mrow = m_ref[hh, u, 0:1, :]
            hrows = _ds(hb * DH, DH, DH)
        m = l = acc = None
        for c in range(NC):
            if hb is not None:
                p = jnp.exp2(s_ref[hh, u, c * KC:(c + 1) * KC, :] - mrow)
                for a in reversed(range(KC // 16)):
                    pr = p[16 * a:16 * a + 8, :] + p[16 * a + 8:16 * a + 16, :]
                    l = pr if l is None else l + pr
                pb = p.astype(bf16)
            if ha is not None:
                kc = k_ref[ga, c * KC:(c + 1) * KC, :]
                s = lax.dot_general(kc, qm, (((1,), (1,)), ((), ())), preferred_element_type=f32)
                s_ref[hh, u, c * KC:(c + 1) * KC, :] = s
                for r in range(KC // 8):
                    sr = s[8 * r:8 * r + 8, :]
                    m = sr if m is None else jnp.maximum(m, sr)
            if hb is not None:
                per = T // KC
                vt = vt_ref[c // per, hrows, (c % per) * KC:(c % per + 1) * KC]
                o = jnp.dot(vt, pb, preferred_element_type=f32)
                acc = o if acc is None else o + acc
            if c + 1 < NC:
                yield
        if ha is not None:
            m_ref[hh, u] = jnp.broadcast_to(jnp.max(m, axis=0, keepdims=True), (8, SUB))
        if hb is not None:
            lsum = jnp.sum(l, axis=0, keepdims=True)
            o = (acc * (1.0 / lsum)).astype(bf16)
            per = SUB // T
            for i in range(per):
                ot_ref[u * per + i, hrows, :] = o[:, i * T:(i + 1) * T]
        yield

    for hh in range(HB):
        for u in range(NS):
            _drain(attn_gen(None, hh, hh, u))

    def head_body(i, carry):
        for hh in range(HB):
            for u in range(NS):
                _drain(attn_gen(i * HB + hh, (i + 1) * HB + hh, hh, u))
        return carry

    lax.fori_loop(0, H // HB - 1, head_body, 0)

    def ln2_gen(t, slot):
        for r in range(0, T, RB):
            hb_ = h_ref[_ds(t * T + r, RB, RB), :]
            y_ref[slot, r:r + RB, :] = _layernorm_centered(_layernorm(hb_)).astype(bf16)
            yield

    def wo_first(t):
        o = ot_ref[t, 0:KP, :].T
        for n in range(D // 128):
            cols = slice(n * 128, (n + 1) * 128)
            a = jnp.dot(o[:, 0:512], wo_ref[0:512, cols], preferred_element_type=f32)
            yield
            a = jnp.dot(o[:, 512:KP], wo_ref[512:KP, cols], preferred_element_type=f32) + a
            h_ref[rows(t), cols] = x_ref[rows(t), cols].astype(f32) + a
            yield

    def wo_rest(t):
        o = ot_ref[t, KP:D, :].T
        for n in range(2):
            cols = slice(n * 512, (n + 1) * 512)
            a = jnp.dot(o, wo_ref[KP:D, cols], preferred_element_type=f32)
            h_ref[rows(t), cols] = a + h_ref[rows(t), cols]
            yield

    def wo_main():
        per = SUB // T
        first = _chain(*[wo_first(t) for t in range(NT)])
        steps = HB * NC
        done = 0
        for u in range(NS):
            target = steps * (u + 1) + 2 * per * u + 3 if u + 1 < NS else 1 << 30
            for _ in first:
                done += 1
                yield
                if done >= target:
                    break
            for _ in _chain(*[wo_rest(u * per + i) for i in range(per)]):
                done += 1
                yield

    wo_copy.wait()
    last_b = _chain(*[attn_gen(H - HB + hh, None, hh, u) for u in range(NS) for hh in range(HB)])
    _interleave(wo_main(), _chain(last_b, ln2_gen(0, 0)), 1)

    w1_copy.wait()
    w2_copy.wait()
    b1_copy.wait()
    b2_copy.wait()

    def mlp_body(t, carry):
        b2 = b2_ref[pl.ds(0, D)].astype(f32).reshape(1, D)
        acc0 = h_ref[rows(t), :] + b2

        def mm1(c):
            z = jnp.dot(y_ref[t & 1], w1_ref[:, c * FC:(c + 1) * FC], preferred_element_type=f32)
            z = z + b1_ref[pl.ds(c * FC, FC)].astype(f32).reshape(1, FC)
            return jax.nn.gelu(z, approximate=True).astype(bf16)

        def chunks():
            acc = acc0
            h1 = mm1(0)
            for c in range(NF):
                w2c = w2_ref[c * FC:(c + 1) * FC, :]
                if c + 1 < NF:
                    h1n = mm1(c + 1)
                    acc = acc + jnp.dot(h1, w2c, preferred_element_type=f32)
                    h1 = h1n
                else:
                    for i in range(T // TO):
                        r = slice(i * TO, (i + 1) * TO)
                        o = acc[r] + jnp.dot(h1[r], w2c, preferred_element_type=f32)
                        o_stage[_ds(t * T + i * TO, TO, TO), :] = o.astype(bf16)
                        out_copy(t * (T // TO) + i).start()
                yield

        _interleave(chunks(), ln2_gen(jnp.minimum(t + 1, NT - 1), (t + 1) & 1), 2)
        return carry

    lax.fori_loop(0, NT, mlp_body, 0)

    pltpu.make_async_copy(o_stage, out_hbm, sems.at[SEM_OUT]).wait()


@jax.jit
def pallas_sequential_preLN__softmax_full_mha__mixer_channel_mlp__prompt_kernel(
    A_x: jax.Array,
    A_wqkv: jax.Array,
    A_wo: jax.Array,
    B_x: jax.Array,
    B_w1: jax.Array,
    B_b1: jax.Array,
    B_w2: jax.Array,
    B_b2: jax.Array,
):
    del B_x
    x = A_x.reshape(S, D)

    any_spec = pl.BlockSpec(memory_space=pl.ANY)
    out = pl.pallas_call(
        _kernel,
        out_shape=jax.ShapeDtypeStruct((S, D), bf16),
        in_specs=[any_spec] * 7,
        out_specs=any_spec,
        scratch_shapes=[
            pltpu.VMEM((S, D), bf16),
            pltpu.VMEM((D, 3 * D), bf16),
            pltpu.VMEM((D, D), bf16),
            pltpu.VMEM((D, F), bf16),
            pltpu.VMEM((BIAS_PAD,), bf16),
            pltpu.VMEM((F, D), bf16),
            pltpu.VMEM((BIAS_PAD,), bf16),
            pltpu.VMEM((T1, D), bf16),
            pltpu.VMEM((G, S, 128), bf16),
            pltpu.VMEM((G, S, 128), bf16),
            pltpu.VMEM((NT, D, T), bf16),
            pltpu.VMEM((HB, NS, S, SUB), f32),
            pltpu.VMEM((HB, NS, 8, SUB), f32),
            pltpu.VMEM((NT, D, T), bf16),
            pltpu.VMEM((2, T, D), bf16),
            pltpu.VMEM((S, D), f32),
            pltpu.VMEM((S, D), bf16),
            pltpu.SemaphoreType.DMA((NSEM,)),
        ],
        compiler_params=pltpu.CompilerParams(vmem_limit_bytes=120 * 1024 * 1024),
    )(x, A_wqkv, A_wo, B_w1, B_b1, B_w2, B_b2)
    return out.reshape(1, S, D)
```
